```python
import os as _os
_os.environ.setdefault("JAX_PLATFORMS", "cpu")
import jax
import jax.numpy as jnp

def _softmax(x, axis=-1):
    return jax.nn.softmax(x, axis=axis)
def _gelu(x):
    return jax.nn.gelu(x, approximate=True)
def _silu(x):
    return jax.nn.silu(x)
def _sigmoid(x):
    return jax.nn.sigmoid(x)
def _layernorm(x, axis=-1, eps=1e-5):
    m = jnp.mean(x, axis=axis, keepdims=True)
    v = jnp.var(x, axis=axis, keepdims=True)
    return (x - m) / jnp.sqrt(v + eps)
def _scatter_add(tgt, idx, src, axis=0):
    return tgt.at[idx].add(src)
def _segment_sum(src, seg, n):
    return jax.ops.segment_sum(src, seg, n)
class _Rng:
    def __init__(self, key):
        self._k = key
    def _next(self):
        self._k, sub = jax.random.split(self._k)
        return sub
    def normal(self, shape):
        return jax.random.normal(self._next(), shape, dtype=jnp.bfloat16)
    def randint(self, lo, hi, shape):
        return jax.random.randint(self._next(), shape, lo, hi, dtype=jnp.int32)
    def uniform(self, shape, lo=0.0, hi=1.0):
        return jax.random.uniform(self._next(), shape, jnp.bfloat16, lo, hi)
    def permutation(self, n):
        return jax.random.permutation(self._next(), n)


kernel_name = 'sequential_preLN__ssm_conv_h3__mixer_channel_mlp__prompt'

def setup_inputs():
    _rng = _Rng(jax.random.key(int.from_bytes(__import__("os").urandom(4), "little")))
    _w = (lambda a: (lambda t: t.astype(jnp.bfloat16) if jnp.issubdtype(t.dtype, jnp.floating) else t)(jnp.asarray(a)))
    def _A_setup():
        B, S, D = 1, 2048, 448
        ks = 4
        return {
            "q": _w((lambda *s: _rng.normal(s) * 0.05)(B, S, D)),
            "k": _w((lambda *s: _rng.normal(s) * 0.05)(B, S, D)),
            "v": _w((lambda *s: _rng.normal(s) * 0.05)(B, S, D)),
            "shift_k": _w((lambda *s: _rng.normal(s) * 0.05)(D, ks) * 0.5),
            "ssm_k": _w((lambda *s: _rng.normal(s) * 0.05)(D, S) * (1.0 / S ** 0.5)),
            "ssm_D": _w((lambda *s: _rng.normal(s) * 0.05)(D)),
        }
    _A_in = _A_setup()

    def _B_setup():
        B, S, D, F = 1, 2048, 448, 1792
        return {
            "x": _w((lambda *s: _rng.normal(s) * 0.05)(B, S, D)),
            "w1": _w((lambda *s: _rng.normal(s) * 0.2)(D, F) * (D ** -0.5)),
            "b1": _w((lambda *s: _rng.normal(s) * 0.2)(F)),
            "w2": _w((lambda *s: _rng.normal(s) * 0.2)(F, D) * (F ** -0.5)),
            "b2": _w((lambda *s: _rng.normal(s) * 0.05)(D)),
        }
    _B_in = _B_setup()

    return {
        "A_q": _A_in["q"],
        "A_k": _A_in["k"],
        "A_v": _A_in["v"],
        "A_shift_k": _A_in["shift_k"],
        "A_ssm_k": _A_in["ssm_k"],
        "A_ssm_D": _A_in["ssm_D"],
        "B_x": _B_in["x"],
        "B_w1": _B_in["w1"],
        "B_b1": _B_in["b1"],
        "B_w2": _B_in["w2"],
        "B_b2": _B_in["b2"],
    }

def reference(A_q, A_k, A_v, A_shift_k, A_ssm_k, A_ssm_D, B_x, B_w1, B_b1, B_w2, B_b2):
    def _A_ref(q, k, v, shift_k, ssm_k, ssm_D):
        B, S, D = q.shape
        ks = shift_k.shape[-1]
        k_pad = jnp.pad(k, ((0, 0), (ks - 1, 0), (0, 0)))
        k_shift = jnp.zeros_like(k)
        for t in range(ks):
            k_shift = k_shift + k_pad[:, t:t + S, :] * shift_k[:, ks - 1 - t][None, None, :]
        kv = k_shift * v
        L = 2 * S
        kv_pad = jnp.pad(kv, ((0, 0), (0, S), (0, 0)))
        kf_pad = jnp.pad(ssm_k, ((0, 0), (0, S)))
        kv_f = (lambda x, axes=(-2,-1): jnp.fft.rfft2(x.astype(jnp.float32), axes=axes))(kv_pad[:, None, :, :], axes=(1, 2))
        kf_f = (lambda x, axes=(-2,-1): jnp.fft.rfft2(x.astype(jnp.float32), axes=axes))(kf_pad[:, None, :], axes=(1, 2))
        kf_f = (lambda x, *d: x.transpose(*d))(kf_f, 1, 2, 0)
        y_f = kv_f * kf_f[None, :, :, :]
        y = (lambda x, s, axes=(-2,-1): jnp.fft.irfft2(x, s=s, axes=axes).astype(jnp.bfloat16))(y_f, (1, L), axes=(1, 2))[:, 0, :S, :]
        y = y + kv * ssm_D[None, None, :]
        return q * y

    def _B_ref(x, w1, b1, w2, b2):
        y = _layernorm(x, axis=-1)
        h = _gelu(jnp.einsum("bsd,df->bsf", y, w1) + b1)
        return jnp.einsum("bsf,fd->bsd", h, w2) + b2

    x = A_q
    h = x + _A_ref(_layernorm(x, axis=-1), A_k, A_v, A_shift_k, A_ssm_k, A_ssm_D)
    h2 = h + _B_ref(_layernorm(h, axis=-1), B_w1, B_b1, B_w2, B_b2)
    return h2
```

```python
import numpy as np
import jax
import jax.numpy as jnp
from jax import lax
import jax.experimental.pallas as pl
import jax.experimental.pallas.tpu as pltpu

_C = 128
_NB = 2
_T = _C * _NB
_EPS = 1e-5


def _dft_matrices():
    f = np.concatenate([np.arange(0, _C, 2), np.arange(1, _C, 2)])
    n = np.arange(_C)
    ang = 2.0 * np.pi * (f[:, None] + 0.5) * n[None, :] / (2 * _C)
    fwd = np.concatenate([np.cos(ang), -np.sin(ang)], axis=0)
    inv = fwd.T / _C
    return fwd.astype(jnp.bfloat16), inv.astype(jnp.bfloat16)


def _layernorm(x):
    m = jnp.mean(x, axis=-1, keepdims=True)
    c = x - m
    v = jnp.mean(c * c, axis=-1, keepdims=True)
    return c * lax.rsqrt(v + _EPS)


def _gelu(x):
    c1 = float(np.sqrt(2.0 / np.pi))
    c2 = c1 * 0.044715
    hx = 0.5 * x
    return hx * jnp.tanh(x * (x * x * c2 + c1)) + hx


def _kernel(q_ref, k_ref, v_ref, sk_ref, ssm_ref, sd_ref, w1_ref, b1_ref, w2_ref,
            b2_ref, fwd_ref, inv_ref, o_ref,
            u_scr, kf_scr, kprev_scr, kpad_scr, kv_scr, z_scr, h_scr, *, n_steps):
    step = pl.program_id(0)
    f32, bf16 = jnp.float32, jnp.bfloat16
    H = _C // 2

    def conv(i):
        if i == 0:
            kpad_scr[0:8, :] = jnp.zeros((8, kpad_scr.shape[1]), f32)
        else:
            kpad_scr[0:8, :] = kpad_scr[_T:_T + 8, :]
        kpad_scr[8:_T + 8, :] = k_ref[...].astype(f32)
        sk = sk_ref[...].astype(f32)
        ks = kpad_scr[8:_T + 8, :] * sk[0:1, :]
        for j in range(1, 4):
            ks = ks + kpad_scr[8 - j:_T + 8 - j, :] * sk[j:j + 1, :]
        kv = ks * v_ref[...].astype(f32)
        kv_scr[...] = kv
        kvb = kv.astype(bf16)
        fwd = fwd_ref[...]
        for b in range(_NB):
            a = i * _NB + b
            u = jnp.dot(fwd, kvb[b * _C:(b + 1) * _C, :], preferred_element_type=f32)
            u_scr[a, 0] = u[:_C]
            u_scr[a, 1] = u[_C:]
            u_scr[a, 2] = u[:_C] + u[_C:]
            kf = lax.dot_general(fwd, ssm_ref[:, b * _C:(b + 1) * _C],
                                 (((1,), (1,)), ((), ())), preferred_element_type=f32)
            kr, ki = kf[:_C], kf[_C:]
            if a > 0:
                pr, pi = kprev_scr[0], kprev_scr[1]
                kr2 = jnp.concatenate([kr[:H] - pi[:H], kr[H:] + pi[H:]], axis=0)
                ki2 = jnp.concatenate([ki[:H] + pr[:H], ki[H:] - pr[H:]], axis=0)
            else:
                kr2, ki2 = kr, ki
            kprev_scr[0] = kr
            kprev_scr[1] = ki
            kf_scr[a, 0] = kr2
            kf_scr[a, 1] = ki2 - kr2
            kf_scr[a, 2] = ki2 + kr2
        a0 = i * _NB
        for r in range(_C // 8):
            rows = slice(r * 8, r * 8 + 8)
            acc = [[None] * 3 for _ in range(_NB)]
            kcache = {}
            for ap in range(a0 + _NB):
                ua = [u_scr[ap, c, rows, :] for c in range(3)]
                for b in range(_NB):
                    m = a0 + b - ap
                    if m < 0:
                        continue
                    if m not in kcache:
                        kcache[m] = [kf_scr[m, c, rows, :] for c in range(3)]
                    kc = kcache[m]
                    p = (kc[0] * ua[2], kc[1] * ua[0], kc[2] * ua[1])
                    for c in range(3):
                        acc[b][c] = p[c] if acc[b][c] is None else acc[b][c] + p[c]
            for b in range(_NB):
                z_scr[b, r * 8:r * 8 + 8, :] = acc[b][0] - acc[b][2]
                z_scr[b, _C + r * 8:_C + r * 8 + 8, :] = acc[b][0] + acc[b][1]
        inv = inv_ref[...]
        sd = sd_ref[...].astype(f32)
        for b in range(_NB):
            rows = slice(b * _C, (b + 1) * _C)
            y = jnp.dot(inv, z_scr[b].astype(bf16), preferred_element_type=f32)
            y = y + kv_scr[rows, :] * sd
            x = q_ref[rows, :].astype(f32)
            h_scr[i % 2, rows, :] = x + _layernorm(x) * y

    def mlp(i):
        h = h_scr[i % 2]
        yn = _layernorm(h).astype(bf16)
        a1 = jnp.dot(yn, w1_ref[...], preferred_element_type=f32) + b1_ref[...].astype(f32)
        g = _gelu(a1).astype(bf16)
        o = jnp.dot(g, w2_ref[...], preferred_element_type=f32)
        o_ref[...] = (h + o + b2_ref[...].astype(f32)).astype(o_ref.dtype)

    for i in range(n_steps + 1):
        @pl.when(step == i)
        def _(i=i):
            if i < n_steps:
                conv(i)
            if i > 0:
                mlp(i - 1)


@jax.jit
def pallas_sequential_preLN__ssm_conv_h3__mixer_channel_mlp__prompt_kernel(
    A_q, A_k, A_v, A_shift_k, A_ssm_k, A_ssm_D, B_x, B_w1, B_b1, B_w2, B_b2,
):
    del B_x
    _, S, D = A_q.shape
    F = B_w1.shape[1]
    n = S // _T
    nblk = S // _C
    fwd, inv = _dft_matrices()
    cur = lambda i: (jnp.minimum(i, n - 1), 0)
    const = lambda i: (0, 0)
    tok = pl.BlockSpec((_T, D), cur)
    full = lambda shape: pl.BlockSpec(shape, const)
    f32 = jnp.float32
    import functools
    out = pl.pallas_call(
        functools.partial(_kernel, n_steps=n),
        grid=(n + 1,),
        in_specs=[tok, tok, tok, full((4, D)),
                  pl.BlockSpec((D, _T), lambda i: (0, jnp.minimum(i, n - 1))),
                  full((1, D)), full((D, F)), full((1, F)), full((F, D)), full((1, D)),
                  full((2 * _C, _C)), full((_C, 2 * _C))],
        out_specs=pl.BlockSpec((_T, D), lambda i: (jnp.maximum(i - 1, 0), 0)),
        out_shape=jax.ShapeDtypeStruct((S, D), A_q.dtype),
        scratch_shapes=[
            pltpu.VMEM((nblk, 3, _C, D), f32),
            pltpu.VMEM((nblk, 3, _C, D), f32),
            pltpu.VMEM((2, _C, D), f32),
            pltpu.VMEM((_T + 8, D), f32),
            pltpu.VMEM((_T, D), f32),
            pltpu.VMEM((_NB, 2 * _C, D), f32),
            pltpu.VMEM((2, _T, D), f32),
        ],
        compiler_params=pltpu.CompilerParams(
            dimension_semantics=("arbitrary",), vmem_limit_bytes=100 * 1024 * 1024),
    )(A_q[0], A_k[0], A_v[0], A_shift_k.T, A_ssm_k, A_ssm_D[None], B_w1, B_b1[None],
      B_w2, B_b2[None], fwd, inv)
    return out[None]
```

```python
import functools

import numpy as np
import jax
import jax.numpy as jnp
from jax import lax
import jax.experimental.pallas as pl
import jax.experimental.pallas.tpu as pltpu

_C = 128
_NB = 2
_T = _C * _NB
_G = 7
_EPS = 1e-5


def _dft_matrices():
    f = np.arange(_C)
    n = np.arange(_C)
    ang = 2.0 * np.pi * n[:, None] * (f[None, :] + 0.5) / (2 * _C)
    fwd = np.concatenate([np.cos(ang), -np.sin(ang)], axis=1)
    inv = fwd.T / _C
    return fwd.astype(jnp.bfloat16), inv.astype(jnp.bfloat16)


def _layernorm(x):
    m = jnp.mean(x, axis=0, keepdims=True)
    c = x - m
    v = jnp.mean(c * c, axis=0, keepdims=True)
    return c * lax.rsqrt(v + _EPS)


def _gelu(x):
    c1 = float(np.sqrt(2.0 / np.pi))
    c2 = c1 * 0.044715
    hx = 0.5 * x
    return hx * jnp.tanh(x * (x * x * c2 + c1)) + hx


def _kernel(q_ref, k_ref, v_ref, sk_ref, ssm_ref, sd_ref, w1_ref, b1_ref, w2_ref,
            b2_ref, fwd_ref, inv_ref, o_ref,
            u_scr, kf_scr, kprev_scr, klast_scr, kv_scr, z_scr, h_scr, yn_scr,
            acc_scr, w1t_scr, par_scr, *, n_steps):
    step = pl.program_id(0)
    f32, bf16 = jnp.float32, jnp.bfloat16
    D = q_ref.shape[0]
    F = w1_ref.shape[1]
    DP = w1t_scr.shape[1]
    RC = D // _G

    @pl.when(step == 0)
    def _init():
        par = jnp.concatenate(
            [sk_ref[...].astype(f32), sd_ref[...].astype(f32), b2_ref[...].astype(f32),
             jnp.zeros((2, D), f32)], axis=0)
        par = jnp.concatenate([par, jnp.zeros((8, DP - D), f32)], axis=1)
        for j in range(6):
            par_scr[j] = jnp.broadcast_to(par[j:j + 1, :], (_C, DP)).T[:D]
        tail = jnp.concatenate(
            [b1_ref[...].astype(f32), jnp.zeros((DP - D - 1, F), f32)], axis=0).astype(bf16)
        for c in range(F // _C):
            cols = slice(c * _C, (c + 1) * _C)
            w = jnp.concatenate([w1_ref[:, cols], tail[:, cols]], axis=0)
            w1t_scr[cols, :] = w.T
        one = (lax.broadcasted_iota(jnp.int32, (DP - D, _T), 0) == 0).astype(bf16)
        yn_scr[D:, :] = one
        klast_scr[...] = jnp.zeros(klast_scr.shape, f32)
        kprev_scr[...] = jnp.zeros(kprev_scr.shape, f32)

    def pre(i):
        kc = k_ref[...].astype(f32)
        kx = jnp.concatenate([klast_scr[...], kc], axis=1)
        klast_scr[...] = kc[:, _T - _C:]
        tile = lambda p: jnp.concatenate([p] * _NB, axis=1)
        ks = kc * tile(par_scr[0])
        for j in range(1, 4):
            ks = ks + pltpu.roll(kx, j, 1)[:, _C:] * tile(par_scr[j])
        kv = ks * v_ref[...].astype(f32)
        kv_scr[...] = kv
        kvb = kv.astype(bf16)
        fwd = fwd_ref[...]
        sgn = (1 - 2 * (lax.broadcasted_iota(jnp.int32, (8, _C), 1) & 1)).astype(f32)
        sgn = jnp.broadcast_to(sgn[0:1], (D, _C))
        for b in range(_NB):
            a = i * _NB + b
            cols = slice(b * _C, (b + 1) * _C)
            u = jnp.dot(kvb[:, cols], fwd, preferred_element_type=f32)
            u_scr[a, 0] = u[:, :_C]
            u_scr[a, 1] = u[:, _C:]
            u_scr[a, 2] = u[:, :_C] + u[:, _C:]
            kf = jnp.dot(ssm_ref[:, cols], fwd, preferred_element_type=f32)
            kr, ki = kf[:, :_C], kf[:, _C:]
            kr2 = kr - sgn * kprev_scr[1]
            ki2 = ki + sgn * kprev_scr[0]
            kprev_scr[0] = kr
            kprev_scr[1] = ki
            kf_scr[a, 0] = kr2
            kf_scr[a, 1] = ki2 - kr2
            kf_scr[a, 2] = ki2 + kr2

    def mac(i, g):
        a0 = i * _NB
        for r in range(RC // 8):
            rows = pl.ds(pl.multiple_of(g * RC + r * 8, 8), 8)
            acc = [[None] * 3 for _ in range(_NB)]
            kcache = {}
            for ap in range(a0 + _NB):
                ua = [u_scr[ap, c, rows, :] for c in range(3)]
                for b in range(_NB):
                    m = a0 + b - ap
                    if m < 0:
                        continue
                    if m not in kcache:
                        kcache[m] = [kf_scr[m, c, rows, :] for c in range(3)]
                    kc = kcache[m]
                    p = (kc[0] * ua[2], kc[1] * ua[0], kc[2] * ua[1])
                    for c in range(3):
                        acc[b][c] = p[c] if acc[b][c] is None else acc[b][c] + p[c]
            for b in range(_NB):
                z_scr[b, rows, 0:_C] = acc[b][0] - acc[b][2]
                z_scr[b, rows, _C:] = acc[b][0] + acc[b][1]

    def mlp(g):
        fs = pl.ds(pl.multiple_of(g * (F // _G), _C), F // _G)
        a1 = jnp.dot(w1t_scr[fs, :], yn_scr[...], preferred_element_type=f32)
        act = _gelu(a1).astype(bf16)
        acc_scr[...] += jnp.dot(w2_ref[:, fs], act, preferred_element_type=f32)

    def post():
        inv = inv_ref[...]
        for b in range(_NB):
            cols = slice(b * _C, (b + 1) * _C)
            y = jnp.dot(z_scr[b].astype(bf16), inv, preferred_element_type=f32)
            y = y + kv_scr[:, cols] * par_scr[4]
            x = q_ref[:, cols].astype(f32)
            h = x + _layernorm(x) * y
            yn_scr[0:D, cols] = _layernorm(h).astype(bf16)
            acc_scr[:, cols] = h + par_scr[5]

    @pl.when(step < n_steps)
    def _():
        pre(step)

    for i in range(n_steps + 1):
        @pl.when(step == i)
        def _(i=i):
            def body(g, carry):
                if i < n_steps:
                    mac(i, g)
                if i > 0:
                    mlp(g)
                return carry
            lax.fori_loop(0, _G, body, 0)

    @pl.when(step > 0)
    def _():
        o_ref[...] = acc_scr[...].astype(o_ref.dtype)

    @pl.when(step < n_steps)
    def _():
        post()


@jax.jit
def pallas_sequential_preLN__ssm_conv_h3__mixer_channel_mlp__prompt_kernel(
    A_q, A_k, A_v, A_shift_k, A_ssm_k, A_ssm_D, B_x, B_w1, B_b1, B_w2, B_b2,
):
    del B_x
    _, S, D = A_q.shape
    F = B_w1.shape[1]
    DP = -(-(D + 1) // _C) * _C
    n = S // _T
    nblk = S // _C
    fwd, inv = _dft_matrices()
    tok = pl.BlockSpec((D, _T), lambda i: (0, jnp.minimum(i, n - 1)))
    full = lambda shape: pl.BlockSpec(shape, lambda i: (0, 0))
    f32, bf16 = jnp.float32, jnp.bfloat16
    out = pl.pallas_call(
        functools.partial(_kernel, n_steps=n),
        grid=(n + 1,),
        in_specs=[tok, tok, tok, full((4, D)), tok,
                  full((1, D)), full((D, F)), full((1, F)), full((D, F)), full((1, D)),
                  full((_C, 2 * _C)), full((2 * _C, _C))],
        out_specs=pl.BlockSpec((D, _T), lambda i: (0, jnp.maximum(i - 1, 0))),
        out_shape=jax.ShapeDtypeStruct((D, S), A_q.dtype),
        scratch_shapes=[
            pltpu.VMEM((nblk, 3, D, _C), f32),
            pltpu.VMEM((nblk, 3, D, _C), f32),
            pltpu.VMEM((2, D, _C), f32),
            pltpu.VMEM((D, _C), f32),
            pltpu.VMEM((D, _T), f32),
            pltpu.VMEM((_NB, D, 2 * _C), f32),
            pltpu.VMEM((8, _C), f32),
            pltpu.VMEM((DP, _T), bf16),
            pltpu.VMEM((D, _T), f32),
            pltpu.VMEM((F, DP), bf16),
            pltpu.VMEM((6, D, _C), f32),
        ],
        compiler_params=pltpu.CompilerParams(
            dimension_semantics=("arbitrary",), vmem_limit_bytes=100 * 1024 * 1024),
    )(A_q[0].T, A_k[0].T, A_v[0].T, A_shift_k.T, A_ssm_k, A_ssm_D[None], B_w1,
      B_b1[None], B_w2.T, B_b2[None], fwd, inv)
    return out.T[None]
```

```python
import functools

import numpy as np
import jax
import jax.numpy as jnp
from jax import lax
import jax.experimental.pallas as pl
import jax.experimental.pallas.tpu as pltpu

_C = 128
_NB = 2
_T = _C * _NB
_G = 7
_EPS = 1e-5


def _dft_matrices():
    f = np.arange(_C)
    n = np.arange(_C)
    ang = 2.0 * np.pi * n[:, None] * (f[None, :] + 0.5) / (2 * _C)
    fwd = np.concatenate([np.cos(ang), -np.sin(ang)], axis=1)
    inv = fwd.T / _C
    return fwd.astype(jnp.bfloat16), inv.astype(jnp.bfloat16)


def _layernorm(x):
    m = jnp.mean(x, axis=0, keepdims=True)
    c = x - m
    v = jnp.mean(c * c, axis=0, keepdims=True)
    return c * lax.rsqrt(v + _EPS)


def _gelu(x):
    c1 = float(np.sqrt(2.0 / np.pi))
    c2 = c1 * 0.044715
    hx = 0.5 * x
    return hx * jnp.tanh(x * (x * x * c2 + c1)) + hx


def _kernel(q_ref, k_ref, v_ref, sk_ref, ssm_ref, sd_ref, w1_ref, b1_ref, w2_ref,
            b2_ref, fwd_ref, inv_ref, o_ref,
            u_scr, kf_scr, kprev_scr, klast_scr, kv_scr, z_scr, h_scr, yn_scr,
            acc_scr, w1t_scr, par_scr, *, n_steps):
    step = pl.program_id(0)
    f32, bf16 = jnp.float32, jnp.bfloat16
    D = q_ref.shape[0]
    F = w1_ref.shape[1]
    DP = w1t_scr.shape[1]
    RC = D // _G

    @pl.when(step == 0)
    def _init():
        par = jnp.concatenate(
            [sk_ref[...].astype(f32), sd_ref[...].astype(f32)[None, :], b2_ref[...].astype(f32)[None, :],
             jnp.zeros((2, D), f32)], axis=0)
        par = jnp.concatenate([par, jnp.zeros((8, DP - D), f32)], axis=1)
        for j in range(6):
            par_scr[j] = jnp.broadcast_to(par[j:j + 1, :], (_C, DP)).T[:D]
        tail = jnp.concatenate(
            [b1_ref[...].astype(f32)[None, :], jnp.zeros((DP - D - 1, F), f32)], axis=0).astype(bf16)
        for c in range(F // _C):
            cols = slice(c * _C, (c + 1) * _C)
            w = jnp.concatenate([w1_ref[:, cols], tail[:, cols]], axis=0)
            w1t_scr[cols, :] = w.T
        one = (lax.broadcasted_iota(jnp.int32, (DP - D, _T), 0) == 0).astype(bf16)
        yn_scr[D:, :] = one
        klast_scr[...] = jnp.zeros(klast_scr.shape, f32)
        kprev_scr[...] = jnp.zeros(kprev_scr.shape, f32)

    def pre(i):
        kc = k_ref[...].astype(f32)
        kx = jnp.concatenate([klast_scr[...], kc], axis=1)
        klast_scr[...] = kc[:, _T - _C:]
        tile = lambda p: jnp.concatenate([p] * _NB, axis=1)
        ks = kc * tile(par_scr[0])
        for j in range(1, 4):
            ks = ks + pltpu.roll(kx, j, 1)[:, _C:] * tile(par_scr[j])
        kv = ks * v_ref[...].astype(f32)
        kv_scr[...] = kv
        kvb = kv.astype(bf16)
        fwd = fwd_ref[...]
        sgn = (1 - 2 * (lax.broadcasted_iota(jnp.int32, (8, _C), 1) & 1)).astype(f32)
        sgn = jnp.broadcast_to(sgn[0:1], (D, _C))
        for b in range(_NB):
            a = i * _NB + b
            cols = slice(b * _C, (b + 1) * _C)
            u = jnp.dot(kvb[:, cols], fwd, preferred_element_type=f32)
            u_scr[a, 0] = u[:, :_C]
            u_scr[a, 1] = u[:, _C:]
            u_scr[a, 2] = u[:, :_C] + u[:, _C:]
            kf = jnp.dot(ssm_ref[:, cols], fwd, preferred_element_type=f32)
            kr, ki = kf[:, :_C], kf[:, _C:]
            kr2 = kr - sgn * kprev_scr[1]
            ki2 = ki + sgn * kprev_scr[0]
            kprev_scr[0] = kr
            kprev_scr[1] = ki
            kf_scr[a, 0] = kr2
            kf_scr[a, 1] = ki2 - kr2
            kf_scr[a, 2] = ki2 + kr2

    def mac(i, g):
        a0 = i * _NB
        for r in range(RC // 8):
            rows = pl.ds(pl.multiple_of(g * RC + r * 8, 8), 8)
            acc = [[None] * 3 for _ in range(_NB)]
            kcache = {}
            for ap in range(a0 + _NB):
                ua = [u_scr[ap, c, rows, :] for c in range(3)]
                for b in range(_NB):
                    m = a0 + b - ap
                    if m < 0:
                        continue
                    if m not in kcache:
                        kcache[m] = [kf_scr[m, c, rows, :] for c in range(3)]
                    kc = kcache[m]
                    p = (kc[0] * ua[2], kc[1] * ua[0], kc[2] * ua[1])
                    for c in range(3):
                        acc[b][c] = p[c] if acc[b][c] is None else acc[b][c] + p[c]
            for b in range(_NB):
                z_scr[b, rows, 0:_C] = acc[b][0] - acc[b][2]
                z_scr[b, rows, _C:] = acc[b][0] + acc[b][1]

    def mlp(g):
        fs = pl.ds(pl.multiple_of(g * (F // _G), _C), F // _G)
        a1 = jnp.dot(w1t_scr[fs, :], yn_scr[...], preferred_element_type=f32)
        act = _gelu(a1).astype(bf16)
        acc_scr[...] += jnp.dot(w2_ref[:, fs], act, preferred_element_type=f32)

    def post():
        inv = inv_ref[...]
        for b in range(_NB):
            cols = slice(b * _C, (b + 1) * _C)
            y = jnp.dot(z_scr[b].astype(bf16), inv, preferred_element_type=f32)
            y = y + kv_scr[:, cols] * par_scr[4]
            x = q_ref[:, cols].astype(f32)
            h = x + _layernorm(x) * y
            yn_scr[0:D, cols] = _layernorm(h).astype(bf16)
            acc_scr[:, cols] = h + par_scr[5]

    @pl.when(step < n_steps)
    def _():
        pre(step)

    for i in range(n_steps + 1):
        @pl.when(step == i)
        def _(i=i):
            def body(g, carry):
                if i < n_steps:
                    mac(i, g)
                if i > 0:
                    mlp(g)
                return carry
            lax.fori_loop(0, _G, body, 0)

    @pl.when(step > 0)
    def _():
        o_ref[...] = acc_scr[...].astype(o_ref.dtype)

    @pl.when(step < n_steps)
    def _():
        post()


@jax.jit
def pallas_sequential_preLN__ssm_conv_h3__mixer_channel_mlp__prompt_kernel(
    A_q, A_k, A_v, A_shift_k, A_ssm_k, A_ssm_D, B_x, B_w1, B_b1, B_w2, B_b2,
):
    del B_x
    _, S, D = A_q.shape
    F = B_w1.shape[1]
    DP = -(-(D + 1) // _C) * _C
    n = S // _T
    nblk = S // _C
    fwd, inv = _dft_matrices()
    tok = pl.BlockSpec((D, _T), lambda i: (0, jnp.minimum(i, n - 1)))
    full = lambda shape: pl.BlockSpec(shape, lambda i: (0, 0))
    vec = lambda m: pl.BlockSpec((m,), lambda i: (0,))
    f32, bf16 = jnp.float32, jnp.bfloat16
    out = pl.pallas_call(
        functools.partial(_kernel, n_steps=n),
        grid=(n + 1,),
        in_specs=[tok, tok, tok, full((4, D)), tok,
                  vec(D), full((D, F)), vec(F), full((D, F)), vec(D),
                  full((_C, 2 * _C)), full((2 * _C, _C))],
        out_specs=pl.BlockSpec((D, _T), lambda i: (0, jnp.maximum(i - 1, 0))),
        out_shape=jax.ShapeDtypeStruct((D, S), A_q.dtype),
        scratch_shapes=[
            pltpu.VMEM((nblk, 3, D, _C), f32),
            pltpu.VMEM((nblk, 3, D, _C), f32),
            pltpu.VMEM((2, D, _C), f32),
            pltpu.VMEM((D, _C), f32),
            pltpu.VMEM((D, _T), f32),
            pltpu.VMEM((_NB, D, 2 * _C), f32),
            pltpu.VMEM((8, _C), f32),
            pltpu.VMEM((DP, _T), bf16),
            pltpu.VMEM((D, _T), f32),
            pltpu.VMEM((F, DP), bf16),
            pltpu.VMEM((6, D, _C), f32),
        ],
        compiler_params=pltpu.CompilerParams(
            dimension_semantics=("arbitrary",), vmem_limit_bytes=100 * 1024 * 1024),
    )(A_q[0].T, A_k[0].T, A_v[0].T, A_shift_k.T, A_ssm_k, A_ssm_D, B_w1,
      B_b1, B_w2.T, B_b2, fwd, inv)
    return out.T[None]
```

```python
import functools

import numpy as np
import jax
import jax.numpy as jnp
from jax import lax
import jax.experimental.pallas as pl
import jax.experimental.pallas.tpu as pltpu

_C = 128
_NB = 2
_T = _C * _NB
_G = 7
_EPS = 1e-5


def _dft_matrices():
    f = np.arange(_C)
    n = np.arange(_C)
    ang = 2.0 * np.pi * n[:, None] * (f[None, :] + 0.5) / (2 * _C)
    fwd = np.concatenate([np.cos(ang), -np.sin(ang)], axis=1)
    inv = fwd.T / _C
    return fwd.astype(jnp.bfloat16), inv.astype(jnp.bfloat16)


def _layernorm(x):
    m = jnp.mean(x, axis=0, keepdims=True)
    c = x - m
    v = jnp.mean(c * c, axis=0, keepdims=True)
    return c * lax.rsqrt(v + _EPS)


def _gelu(x):
    c1 = float(np.sqrt(2.0 / np.pi))
    c2 = c1 * 0.044715
    hx = 0.5 * x
    return hx * jnp.tanh(x * (x * x * c2 + c1)) + hx


def _kernel(q_ref, k_ref, v_ref, sk_ref, ssm_ref, sd_ref, w1_ref, b1_ref, w2_ref,
            b2_ref, fwd_ref, inv_ref, o_ref,
            u_scr, kf_scr, kprev_scr, klast_scr, kv_scr, z_scr, h_scr, yn_scr,
            acc_scr, w1t_scr, par_scr, *, n_steps):
    step = pl.program_id(0)
    f32, bf16 = jnp.float32, jnp.bfloat16
    D = q_ref.shape[0]
    F = w1_ref.shape[1]
    DP = w1t_scr.shape[1]
    RC = D // _G

    @pl.when(step == 0)
    def _init():
        par = jnp.concatenate(
            [sk_ref[...].astype(f32), sd_ref[...].astype(f32)[None, :], b2_ref[...].astype(f32)[None, :],
             jnp.zeros((2, D), f32)], axis=0)
        par = jnp.concatenate([par, jnp.zeros((8, DP - D), f32)], axis=1)
        for j in range(6):
            par_scr[j] = jnp.broadcast_to(par[j:j + 1, :], (_C, DP)).T[:D]
        tail = jnp.concatenate(
            [b1_ref[...].astype(f32)[None, :], jnp.zeros((DP - D - 1, F), f32)], axis=0).astype(bf16)
        for c in range(F // _C):
            cols = slice(c * _C, (c + 1) * _C)
            w = jnp.concatenate([w1_ref[:, cols], tail[:, cols]], axis=0)
            w1t_scr[cols, :] = w.T
        one = (lax.broadcasted_iota(jnp.int32, (DP - D, _T), 0) == 0).astype(bf16)
        yn_scr[D:, :] = one
        klast_scr[...] = jnp.zeros(klast_scr.shape, f32)
        kprev_scr[...] = jnp.zeros(kprev_scr.shape, f32)

    def pre(i):
        kc = k_ref[...].astype(f32)
        kx = jnp.concatenate([klast_scr[...], kc], axis=1)
        klast_scr[...] = kc[:, _T - _C:]
        tile = lambda p: jnp.concatenate([p] * _NB, axis=1)
        ks = kc * tile(par_scr[0])
        for j in range(1, 4):
            ks = ks + pltpu.roll(kx, j, 1)[:, _C:] * tile(par_scr[j])
        kv = ks * v_ref[...].astype(f32)
        kv_scr[...] = kv
        kvb = kv.astype(bf16)
        fwd = fwd_ref[...]
        sgn = (1 - 2 * (lax.broadcasted_iota(jnp.int32, (8, _C), 1) & 1)).astype(f32)
        sgn = jnp.broadcast_to(sgn[0:1], (D, _C))
        for b in range(_NB):
            a = i * _NB + b
            cols = slice(b * _C, (b + 1) * _C)
            u = jnp.dot(kvb[:, cols], fwd, preferred_element_type=f32)
            u_scr[a, 0] = u[:, :_C]
            u_scr[a, 1] = u[:, _C:]
            u_scr[a, 2] = u[:, :_C] + u[:, _C:]
            kf = jnp.dot(ssm_ref[:, cols], fwd, preferred_element_type=f32)
            kr, ki = kf[:, :_C], kf[:, _C:]
            kr2 = kr - sgn * kprev_scr[1]
            ki2 = ki + sgn * kprev_scr[0]
            kprev_scr[0] = kr
            kprev_scr[1] = ki
            kf_scr[a, 0] = kr2
            kf_scr[a, 1] = ki2 - kr2
            kf_scr[a, 2] = ki2 + kr2

    def mac(i, g, rs):
        a0 = i * _NB
        for r in rs:
            rows = pl.ds(pl.multiple_of(g * RC + r * 8, 8), 8)
            acc = [[None] * 3 for _ in range(_NB)]
            kcache = {}
            for ap in range(a0 + _NB):
                ua = [u_scr[ap, c, rows, :] for c in range(3)]
                for b in range(_NB):
                    m = a0 + b - ap
                    if m < 0:
                        continue
                    if m not in kcache:
                        kcache[m] = [kf_scr[m, c, rows, :] for c in range(3)]
                    kc = kcache[m]
                    p = (kc[0] * ua[2], kc[1] * ua[0], kc[2] * ua[1])
                    for c in range(3):
                        acc[b][c] = p[c] if acc[b][c] is None else acc[b][c] + p[c]
            for b in range(_NB):
                z_scr[b, rows, 0:_C] = acc[b][0] - acc[b][2]
                z_scr[b, rows, _C:] = acc[b][0] + acc[b][1]

    FC = F // _G

    def post():
        inv = inv_ref[...]
        for b in range(_NB):
            cols = slice(b * _C, (b + 1) * _C)
            y = jnp.dot(z_scr[b].astype(bf16), inv, preferred_element_type=f32)
            y = y + kv_scr[:, cols] * par_scr[4]
            x = q_ref[:, cols].astype(f32)
            h = x + _layernorm(x) * y
            yn_scr[0:D, cols] = _layernorm(h).astype(bf16)
            acc_scr[:, cols] = h + par_scr[5]

    @pl.when(step < n_steps)
    def _():
        pre(step)

    for i in range(n_steps + 1):
        @pl.when(step == i)
        def _(i=i):
            def body(g, carry):
                acts = []
                fs = pl.ds(pl.multiple_of(g * FC, _C), FC)
                dot = functools.partial(jnp.dot, preferred_element_type=f32)
                m = lambda r: mac(i, g, [r]) if i < n_steps else None
                for nb in range(_NB):
                    cols = slice(nb * _C, (nb + 1) * _C)
                    if i > 0:
                        a1 = dot(w1t_scr[fs, :DP // 2], yn_scr[:DP // 2, cols])
                    m(2 * nb)
                    if i > 0:
                        a1 += dot(w1t_scr[fs, DP // 2:], yn_scr[DP // 2:, cols])
                        acts.append(_gelu(a1).astype(bf16))
                    m(2 * nb + 1)
                for nb in range(_NB):
                    cols = slice(nb * _C, (nb + 1) * _C)
                    for kk in range(2):
                        if i > 0:
                            f2 = pl.ds(pl.multiple_of(g * FC + kk * _C, _C), _C)
                            o = dot(w2_ref[:, f2], acts[nb][kk * _C:(kk + 1) * _C])
                            part = o if kk == 0 else part + o
                        m(4 + 2 * nb + kk)
                    if i > 0:
                        acc_scr[:, cols] += part
                return carry
            lax.fori_loop(0, _G, body, 0)

    @pl.when(step > 0)
    def _():
        o_ref[...] = acc_scr[...].astype(o_ref.dtype)

    @pl.when(step < n_steps)
    def _():
        post()


@jax.jit
def pallas_sequential_preLN__ssm_conv_h3__mixer_channel_mlp__prompt_kernel(
    A_q, A_k, A_v, A_shift_k, A_ssm_k, A_ssm_D, B_x, B_w1, B_b1, B_w2, B_b2,
):
    del B_x
    _, S, D = A_q.shape
    F = B_w1.shape[1]
    DP = -(-(D + 1) // _C) * _C
    n = S // _T
    nblk = S // _C
    fwd, inv = _dft_matrices()
    tok = pl.BlockSpec((D, _T), lambda i: (0, jnp.minimum(i, n - 1)))
    full = lambda shape: pl.BlockSpec(shape, lambda i: (0, 0))
    vec = lambda m: pl.BlockSpec((m,), lambda i: (0,))
    f32, bf16 = jnp.float32, jnp.bfloat16
    out = pl.pallas_call(
        functools.partial(_kernel, n_steps=n),
        grid=(n + 1,),
        in_specs=[tok, tok, tok, full((4, D)), tok,
                  vec(D), full((D, F)), vec(F), full((D, F)), vec(D),
                  full((_C, 2 * _C)), full((2 * _C, _C))],
        out_specs=pl.BlockSpec((D, _T), lambda i: (0, jnp.maximum(i - 1, 0))),
        out_shape=jax.ShapeDtypeStruct((D, S), A_q.dtype),
        scratch_shapes=[
            pltpu.VMEM((nblk, 3, D, _C), f32),
            pltpu.VMEM((nblk, 3, D, _C), f32),
            pltpu.VMEM((2, D, _C), f32),
            pltpu.VMEM((D, _C), f32),
            pltpu.VMEM((D, _T), f32),
            pltpu.VMEM((_NB, D, 2 * _C), f32),
            pltpu.VMEM((8, _C), f32),
            pltpu.VMEM((DP, _T), bf16),
            pltpu.VMEM((D, _T), f32),
            pltpu.VMEM((F, DP), bf16),
            pltpu.VMEM((6, D, _C), f32),
        ],
        compiler_params=pltpu.CompilerParams(
            dimension_semantics=("arbitrary",), vmem_limit_bytes=100 * 1024 * 1024),
    )(A_q[0].T, A_k[0].T, A_v[0].T, A_shift_k.T, A_ssm_k, A_ssm_D, B_w1,
      B_b1, B_w2.T, B_b2, fwd, inv)
    return out.T[None]
```

```python
import functools

import numpy as np
import jax
import jax.numpy as jnp
from jax import lax
import jax.experimental.pallas as pl
import jax.experimental.pallas.tpu as pltpu

_C = 128
_NB = 2
_T = _C * _NB
_G = 7
_EPS = 1e-5


def _dft_matrices():
    f = np.arange(_C)
    n = np.arange(_C)
    ang = 2.0 * np.pi * n[:, None] * (f[None, :] + 0.5) / (2 * _C)
    fwd = np.concatenate([np.cos(ang), -np.sin(ang)], axis=1)
    inv = fwd.T / _C
    return fwd.astype(jnp.bfloat16), inv.astype(jnp.bfloat16)


def _layernorm(x):
    m = jnp.mean(x, axis=0, keepdims=True)
    c = x - m
    v = jnp.mean(c * c, axis=0, keepdims=True)
    return c * lax.rsqrt(v + _EPS)


def _gelu(x):
    c1 = float(np.sqrt(2.0 / np.pi))
    c2 = c1 * 0.044715
    hx = 0.5 * x
    return hx * jnp.tanh(x * (x * x * c2 + c1)) + hx


def _kernel(q_ref, k_ref, v_ref, sk_ref, ssm_ref, sd_ref, w1_ref, b1_ref, w2_ref,
            b2_ref, fwd_ref, inv_ref, o_ref,
            u_scr, kf_scr, kprev_scr, klast_scr, kv_scr, z_scr, h_scr, yn_scr,
            acc_scr, w1t_scr, par_scr, *, n_steps):
    step = pl.program_id(0)
    f32, bf16 = jnp.float32, jnp.bfloat16
    D = q_ref.shape[0]
    F = w1_ref.shape[1]
    DP = w1t_scr.shape[1]
    RC = D // _G

    @pl.when(step == 0)
    def _init():
        par = jnp.concatenate(
            [sk_ref[...].astype(f32), sd_ref[...].astype(f32)[None, :], b2_ref[...].astype(f32)[None, :],
             jnp.zeros((2, D), f32)], axis=0)
        par = jnp.concatenate([par, jnp.zeros((8, DP - D), f32)], axis=1)
        for j in range(6):
            par_scr[j] = jnp.broadcast_to(par[j:j + 1, :], (_C, DP)).T[:D]
        tail = jnp.concatenate(
            [b1_ref[...].astype(f32)[None, :], jnp.zeros((DP - D - 1, F), f32)], axis=0).astype(bf16)
        for c in range(F // _C):
            cols = slice(c * _C, (c + 1) * _C)
            w = jnp.concatenate([w1_ref[:, cols], tail[:, cols]], axis=0)
            w1t_scr[cols, :] = w.T
        one = (lax.broadcasted_iota(jnp.int32, (DP - D, _T), 0) == 0).astype(bf16)
        yn_scr[D:, :] = one
        klast_scr[...] = jnp.zeros(klast_scr.shape, f32)
        kprev_scr[...] = jnp.zeros(kprev_scr.shape, f32)

    def pre(i):
        kc = k_ref[...].astype(f32)
        kx = jnp.concatenate([klast_scr[...], kc], axis=1)
        klast_scr[...] = kc[:, _T - _C:]
        tile = lambda p: jnp.concatenate([p] * _NB, axis=1)
        ks = kc * tile(par_scr[0])
        for j in range(1, 4):
            ks = ks + pltpu.roll(kx, j, 1)[:, _C:] * tile(par_scr[j])
        kv = ks * v_ref[...].astype(f32)
        kv_scr[...] = kv
        kvb = kv.astype(bf16)
        fwd = fwd_ref[...]
        sgn = (1 - 2 * (lax.broadcasted_iota(jnp.int32, (8, _C), 1) & 1)).astype(f32)
        sgn = jnp.broadcast_to(sgn[0:1], (D, _C))
        for b in range(_NB):
            a = i * _NB + b
            cols = slice(b * _C, (b + 1) * _C)
            u = jnp.dot(kvb[:, cols], fwd, preferred_element_type=f32)
            u_scr[a, 0] = u[:, :_C]
            u_scr[a, 1] = u[:, _C:]
            u_scr[a, 2] = u[:, :_C] + u[:, _C:]
            kf = jnp.dot(ssm_ref[:, cols], fwd, preferred_element_type=f32)
            kr, ki = kf[:, :_C], kf[:, _C:]
            kr2 = kr - sgn * kprev_scr[1]
            ki2 = ki + sgn * kprev_scr[0]
            kprev_scr[0] = kr
            kprev_scr[1] = ki
            kf_scr[a, 0] = kr2
            kf_scr[a, 1] = ki2 - kr2
            kf_scr[a, 2] = ki2 + kr2

    def mac(i, g, rs, dep):
        a0 = i * _NB
        for r in rs:
            rows = pl.ds(pl.multiple_of(g * RC + r * 8, 8), 8)
            acc = [[None] * 3 for _ in range(_NB)]
            kcache = {}
            for ap in range(a0 + _NB):
                ua = [u_scr[ap, c, rows, :] for c in range(3)]
                for b in range(_NB):
                    m = a0 + b - ap
                    if m < 0:
                        continue
                    if m not in kcache:
                        kcache[m] = [kf_scr[m, c, rows, :] for c in range(3)]
                    kc = kcache[m]
                    p = (kc[0] * ua[2], kc[1] * ua[0], kc[2] * ua[1])
                    for c in range(3):
                        if acc[b][c] is not None:
                            acc[b][c] = acc[b][c] + p[c]
                        elif dep is None:
                            acc[b][c] = p[c]
                        else:
                            acc[b][c] = jnp.where(g >= 0, p[c], dep[:8, :_C])
            for b in range(_NB):
                z_scr[b, rows, 0:_C] = acc[b][0] - acc[b][2]
                z_scr[b, rows, _C:] = acc[b][0] + acc[b][1]

    FC = F // _G

    def post():
        inv = inv_ref[...]
        for b in range(_NB):
            cols = slice(b * _C, (b + 1) * _C)
            y = jnp.dot(z_scr[b].astype(bf16), inv, preferred_element_type=f32)
            y = y + kv_scr[:, cols] * par_scr[4]
            x = q_ref[:, cols].astype(f32)
            h = x + _layernorm(x) * y
            yn_scr[0:D, cols] = _layernorm(h).astype(bf16)
            acc_scr[:, cols] = h + par_scr[5]

    @pl.when(step < n_steps)
    def _():
        pre(step)

    for i in range(n_steps + 1):
        @pl.when(step == i)
        def _(i=i):
            def body(g, carry):
                acts = []
                fs = pl.ds(pl.multiple_of(g * FC, _C), FC)
                dot = functools.partial(jnp.dot, preferred_element_type=f32)
                m = lambda r, d=None: mac(i, g, [r], d) if i < n_steps else None
                for nb in range(_NB):
                    cols = slice(nb * _C, (nb + 1) * _C)
                    if i > 0:
                        a1 = dot(w1t_scr[fs, :DP // 2], yn_scr[:DP // 2, cols])
                    m(2 * nb, acts[0].astype(f32) if acts else None)
                    if i > 0:
                        a1 += dot(w1t_scr[fs, DP // 2:], yn_scr[DP // 2:, cols])
                        acts.append(_gelu(a1).astype(bf16))
                    m(2 * nb + 1, a1 if i else None)
                for nb in range(_NB):
                    cols = slice(nb * _C, (nb + 1) * _C)
                    for kk in range(2):
                        if i > 0:
                            f2 = pl.ds(pl.multiple_of(g * FC + kk * _C, _C), _C)
                            o = dot(w2_ref[:, f2], acts[nb][kk * _C:(kk + 1) * _C])
                            part = o if kk == 0 else part + o
                        m(4 + 2 * nb + kk, o if i and (nb, kk) != (1, 1) else (acts[1].astype(f32) if i else None))
                    if i > 0:
                        acc_scr[:, cols] += part
                return carry
            lax.fori_loop(0, _G, body, 0)

    @pl.when(step > 0)
    def _():
        o_ref[...] = acc_scr[...].astype(o_ref.dtype)

    @pl.when(step < n_steps)
    def _():
        post()


@jax.jit
def pallas_sequential_preLN__ssm_conv_h3__mixer_channel_mlp__prompt_kernel(
    A_q, A_k, A_v, A_shift_k, A_ssm_k, A_ssm_D, B_x, B_w1, B_b1, B_w2, B_b2,
):
    del B_x
    _, S, D = A_q.shape
    F = B_w1.shape[1]
    DP = -(-(D + 1) // _C) * _C
    n = S // _T
    nblk = S // _C
    fwd, inv = _dft_matrices()
    tok = pl.BlockSpec((D, _T), lambda i: (0, jnp.minimum(i, n - 1)))
    full = lambda shape: pl.BlockSpec(shape, lambda i: (0, 0))
    vec = lambda m: pl.BlockSpec((m,), lambda i: (0,))
    f32, bf16 = jnp.float32, jnp.bfloat16
    out = pl.pallas_call(
        functools.partial(_kernel, n_steps=n),
        grid=(n + 1,),
        in_specs=[tok, tok, tok, full((4, D)), tok,
                  vec(D), full((D, F)), vec(F), full((D, F)), vec(D),
                  full((_C, 2 * _C)), full((2 * _C, _C))],
        out_specs=pl.BlockSpec((D, _T), lambda i: (0, jnp.maximum(i - 1, 0))),
        out_shape=jax.ShapeDtypeStruct((D, S), A_q.dtype),
        scratch_shapes=[
            pltpu.VMEM((nblk, 3, D, _C), f32),
            pltpu.VMEM((nblk, 3, D, _C), f32),
            pltpu.VMEM((2, D, _C), f32),
            pltpu.VMEM((D, _C), f32),
            pltpu.VMEM((D, _T), f32),
            pltpu.VMEM((_NB, D, 2 * _C), f32),
            pltpu.VMEM((8, _C), f32),
            pltpu.VMEM((DP, _T), bf16),
            pltpu.VMEM((D, _T), f32),
            pltpu.VMEM((F, DP), bf16),
            pltpu.VMEM((6, D, _C), f32),
        ],
        compiler_params=pltpu.CompilerParams(
            dimension_semantics=("arbitrary",), vmem_limit_bytes=100 * 1024 * 1024),
    )(A_q[0].T, A_k[0].T, A_v[0].T, A_shift_k.T, A_ssm_k, A_ssm_D, B_w1,
      B_b1, B_w2.T, B_b2, fwd, inv)
    return out.T[None]
```
